```python
import os as _os
_os.environ.setdefault("JAX_PLATFORMS", "cpu")
import jax
import jax.numpy as jnp

def _softmax(x, axis=-1):
    return jax.nn.softmax(x, axis=axis)
def _gelu(x):
    return jax.nn.gelu(x, approximate=True)
def _silu(x):
    return jax.nn.silu(x)
def _sigmoid(x):
    return jax.nn.sigmoid(x)
def _layernorm(x, axis=-1, eps=1e-5):
    m = jnp.mean(x, axis=axis, keepdims=True)
    v = jnp.var(x, axis=axis, keepdims=True)
    return (x - m) / jnp.sqrt(v + eps)
def _scatter_add(tgt, idx, src, axis=0):
    return tgt.at[idx].add(src)
def _segment_sum(src, seg, n):
    return jax.ops.segment_sum(src, seg, n)
class _Rng:
    def __init__(self, key):
        self._k = key
    def _next(self):
        self._k, sub = jax.random.split(self._k)
        return sub
    def normal(self, shape):
        return jax.random.normal(self._next(), shape, dtype=jnp.bfloat16)
    def randint(self, lo, hi, shape):
        return jax.random.randint(self._next(), shape, lo, hi, dtype=jnp.int32)
    def uniform(self, shape, lo=0.0, hi=1.0):
        return jax.random.uniform(self._next(), shape, jnp.bfloat16, lo, hi)
    def permutation(self, n):
        return jax.random.permutation(self._next(), n)


kernel_name = 'parallel_sum__ssm_conv_s5__glu_gated_swiglu__prompt'

def setup_inputs():
    _rng = _Rng(jax.random.key(int.from_bytes(__import__("os").urandom(4), "little")))
    _w = (lambda a: (lambda t: t.astype(jnp.bfloat16) if jnp.issubdtype(t.dtype, jnp.floating) else t)(jnp.asarray(a)))
    def _A_setup():
        B, S, D = 1, 2048, 640
        P = D
        Lambda_re = -0.5 * jnp.exp((lambda *s: _rng.normal(s) * 0.4)(P))
        Lambda_im = (lambda *s: _rng.normal(s) * 0.4)(P) * 1.0
        B_re = (lambda *s: _rng.normal(s) * 0.4)(P, D) * (D ** -0.5)
        B_im = (lambda *s: _rng.normal(s) * 0.4)(P, D) * (D ** -0.5)
        C_re = (lambda *s: _rng.normal(s) * 0.4)(D, P) * (P ** -0.5)
        C_im = (lambda *s: _rng.normal(s) * 0.4)(D, P) * (P ** -0.5)
        log_dt = (lambda *s: _rng.normal(s) * 0.4)(P) * 0.3 - 2.0
        Dskip = (lambda *s: _rng.normal(s) * 0.4)(D)
        return {
            "x": _w((lambda *s: _rng.normal(s) * 0.05)(B, S, D)),
            "Lambda_re": _w(Lambda_re),
            "Lambda_im": _w(Lambda_im),
            "B_re": _w(B_re),
            "B_im": _w(B_im),
            "C_re": _w(C_re),
            "C_im": _w(C_im),
            "log_dt": _w(log_dt),
            "Dskip": _w(Dskip),
        }
    _A_in = _A_setup()

    def _B_setup():
        B, S, D, F = 1, 2048, 640, 1728
        return {
            "x": _w((lambda *s: _rng.normal(s) * 0.05)(B, S, D)),
            "w1": _w((lambda *s: _rng.normal(s) * 0.1)(D, F) * (2.0 / D) ** 0.5),
            "w3": _w((lambda *s: _rng.normal(s) * 0.1)(D, F) * (2.0 / D) ** 0.5),
            "w2": _w((lambda *s: _rng.normal(s) * 0.1)(F, D) * (2.0 / F) ** 0.5),
        }
    _B_in = _B_setup()

    return {
        "A_x": _A_in["x"],
        "A_Lambda_re": _A_in["Lambda_re"],
        "A_Lambda_im": _A_in["Lambda_im"],
        "A_B_re": _A_in["B_re"],
        "A_B_im": _A_in["B_im"],
        "A_C_re": _A_in["C_re"],
        "A_C_im": _A_in["C_im"],
        "A_log_dt": _A_in["log_dt"],
        "A_Dskip": _A_in["Dskip"],
        "B_x": _B_in["x"],
        "B_w1": _B_in["w1"],
        "B_w3": _B_in["w3"],
        "B_w2": _B_in["w2"],
    }

def reference(A_x, A_Lambda_re, A_Lambda_im, A_B_re, A_B_im, A_C_re, A_C_im, A_log_dt, A_Dskip, B_x, B_w1, B_w3, B_w2):
    def _A_ref(x, Lambda_re, Lambda_im, B_re, B_im, C_re, C_im, log_dt, Dskip):
        Bsz, L, H = x.shape
        Lam = Lambda_re + 1j * Lambda_im
        Bmat = B_re + 1j * B_im
        Cmat = C_re + 1j * C_im
        dt = jnp.exp(log_dt)
        Lam_bar = jnp.exp(dt * Lam)
        B_bar = ((Lam_bar - 1.0) / Lam)[:, None] * Bmat
        Bu = jnp.einsum("bld,pd->blp", x + 0j, B_bar)
        h = jnp.zeros_like(Bu[:, 0, :])
        hs = []
        for t in range(L):
            h = Lam_bar[None, :] * h + Bu[:, t, :]
            hs.append(h)
        hseq = jnp.stack(hs, 1)
        y = 2.0 * jnp.einsum("blp,dp->bld", hseq, Cmat).real + x * Dskip[None, None, :]
        return y

    def _B_ref(x, w1, w3, w2):
        gate = jnp.einsum("bsd,df->bsf", x, w1)
        up = jnp.einsum("bsd,df->bsf", x, w3)
        h = _silu(gate) * up
        out = jnp.einsum("bsf,fd->bsd", h, w2)
        return out

    x = A_x
    xn = _layernorm(x, axis=-1)
    return x + _A_ref(xn, A_Lambda_re, A_Lambda_im, A_B_re, A_B_im, A_C_re, A_C_im, A_log_dt, A_Dskip) + _B_ref(xn, B_w1, B_w3, B_w2)
```

```python
import jax
import jax.numpy as jnp
from jax import lax
import jax.experimental.pallas as pl
import jax.experimental.pallas.tpu as pltpu

L, D, P, F = 2048, 640, 640, 1728
BLOCKS = (528, 496, 528, 496)
CH = 256
ORDER = 1024
NC = D // 128
FA = 1664
FH = 768
SEGS = sorted(set(t // 8 for t in BLOCKS))
f32 = jnp.float32
bf16 = jnp.bfloat16
NT = (((1,), (1,)), ((), ()))


def _cmul(ar, ai, br, bi):
    return ar * br - ai * bi, ar * bi + ai * br


def _dnt(a, b):
    return lax.dot_general(a, b, NT, preferred_element_type=f32)


def _kernel(lre_ref, lim_ref, ldt_ref, dsk_ref,
            x_hbm, bre_hbm, bim_hbm, cre_hbm, cim_hbm, w1_hbm, w3_hbm, w2_hbm, o_hbm,
            xs_ref, os_ref, bre_ref, bim_ref, cre_ref, cim_ref, w1_ref, w3_ref, wt_ref, w2_ref,
            cp_ref, xn_ref, res_ref, u_ref, g_ref, hh_ref, isem, osem):
    nb = len(BLOCKS)
    offs = [sum(BLOCKS[:b]) for b in range(nb)]
    copies = {}

    def add(key, src, dst):
        k = sum(len(v) for v in copies.values())
        cp = pltpu.make_async_copy(src, dst, isem.at[k])
        cp.start()
        copies.setdefault(key, []).append(cp)

    def wait(key):
        for cp in copies[key]:
            cp.wait()

    def add_x(b):
        r = pl.ds(offs[b], BLOCKS[b])
        for c in range(NC):
            add(("x", b), x_hbm.at[r, pl.ds(128 * c, 128)], xs_ref.at[c, r])

    add_x(0)
    add("bre", bre_hbm, bre_ref)
    add("bim", bim_hbm, bim_ref)
    add("fa", w1_hbm.at[pl.ds(0, FH)], w1_ref.at[pl.ds(0, FH)])
    add("fa", w3_hbm.at[pl.ds(0, FH)], w3_ref.at[pl.ds(0, FH)])
    add("fb", w1_hbm.at[pl.ds(FH, FA - FH)], w1_ref.at[pl.ds(FH, FA - FH)])
    add("fb", w3_hbm.at[pl.ds(FH, FA - FH)], w3_ref.at[pl.ds(FH, FA - FH)])
    add("fb", w1_hbm.at[pl.ds(FA, F - FA)], wt_ref.at[pl.ds(0, F - FA)])
    add("fb", w3_hbm.at[pl.ds(FA, F - FA)], wt_ref.at[pl.ds(F - FA, F - FA)])
    add("c", cre_hbm, cre_ref)
    add("c", cim_hbm, cim_ref)
    add_x(1)
    add("w2", w2_hbm, w2_ref)
    for b in range(2, nb):
        add_x(b)

    lre = lre_ref[...].astype(f32).reshape(1, P)
    lim = lim_ref[...].astype(f32).reshape(1, P)
    dt = jnp.exp(ldt_ref[...].astype(f32).reshape(1, P)).astype(bf16).astype(f32)
    dsk = dsk_ref[...].astype(f32).reshape(1, D)
    mag = jnp.exp(dt * lre)
    ar1 = mag * jnp.cos(dt * lim)
    ai1 = mag * jnp.sin(dt * lim)
    den = lre * lre + lim * lim
    kr = ((ar1 - 1.0) * lre + ai1 * lim) / den
    ki = (ai1 * lre - (ar1 - 1.0) * lim) / den
    p2 = [(ar1, ai1)]
    while (1 << len(p2)) <= SEGS[-1]:
        p2.append(_cmul(*p2[-1], *p2[-1]))
    pows = {}
    for s_ in SEGS:
        acc = None
        for k, pk in enumerate(p2):
            if (s_ >> k) & 1:
                acc = pk if acc is None else _cmul(*acc, *pk)
        for q in range(3):
            pows[s_ << q] = acc
            acc = _cmul(*acc, *acc)
    bc = lambda v: jnp.broadcast_to(v, (8, P))
    ar, ai = bc(ar1), bc(ai1)
    row = lax.broadcasted_iota(jnp.int32, (8, P), 0)
    x32 = xs_ref.bitcast(jnp.uint32)

    def norm(b):
        T, o = BLOCKS[b], offs[b]
        S = T // 8
        for j in range(S // 2):
            w = jnp.concatenate(
                [x32[c, pl.ds(o // 2 + j, 8, stride=S // 2), :] for c in range(NC)], axis=1)
            xns = []
            for par in range(2):
                xv = pltpu.bitcast(w << 16 if par == 0 else w & jnp.uint32(0xFFFF0000), f32)
                m = jnp.mean(xv, axis=-1, keepdims=True)
                xc = xv - m
                v = jnp.mean(xc * xc, axis=-1, keepdims=True)
                xn = xc * lax.rsqrt(v + 1e-5)
                xns.append(xn)
                res_ref[pl.ds(o + 16 * j + 8 * par, 8), :] = xv + xn * dsk
            xn_ref[pl.ds(o + 16 * j, 16), :] = jnp.concatenate(xns, axis=0).astype(bf16)

    def scan(b, cr, ci):
        T, o = BLOCKS[b], offs[b]
        S = T // 8

        def ld(t):
            return u_ref[pl.ds(o + 8 * t, 8), 0:P], u_ref[pl.ds(o + 8 * t, 8), P:2 * P]

        er, ei = ld(0)
        for t in range(1, S):
            ur, ui = ld(t)
            er, ei = ar * er - ai * ei + ur, ar * ei + ai * er + ui
        hr = jnp.where(row == 0, cr, pltpu.roll(er, 1, 0))
        hi = jnp.where(row == 0, ci, pltpu.roll(ei, 1, 0))
        for q in range(3):
            sh = 1 << q
            pr, pi = pows[S * sh]
            sr = jnp.where(row >= sh, pltpu.roll(hr, sh, 0), 0.0)
            si = jnp.where(row >= sh, pltpu.roll(hi, sh, 0), 0.0)
            hr, hi = hr + pr * sr - pi * si, hi + pr * si + pi * sr
        for j in range(S // 2):
            rs, is_ = [], []
            for par in range(2):
                ur, ui = ld(2 * j + par)
                hr, hi = ar * hr - ai * hi + ur, ar * hi + ai * hr + ui
                rs.append(hr)
                is_.append(hi)
            g_ref[pl.ds(o + 16 * j, 16), 0:P] = jnp.concatenate(rs, axis=0).astype(bf16)
            g_ref[pl.ds(o + 16 * j, 16), P:2 * P] = jnp.concatenate(is_, axis=0).astype(bf16)
        return bc(hr[7:8, :]), bc(hi[7:8, :])

    def glu(g, u):
        return (g * jax.nn.sigmoid(g) * u).astype(bf16)

    cr = jnp.zeros((8, P), f32)
    ci = jnp.zeros((8, P), f32)
    outs = []
    wait(("x", 0))
    norm(0)
    wait("bre")
    wait("bim")
    for b in range(nb):
        T, o = BLOCKS[b], offs[b]
        S = T // 8
        r = pl.ds(o, T)
        first = b == 0
        u_ref[r, 0:P] = _dnt(xn_ref[r, :], bre_ref[...])
        u_ref[r, P:2 * P] = _dnt(xn_ref[r, :], bim_ref[...])
        if first:
            wait("fa")
            wait("fb")
        cr, ci = scan(b, cr, ci)
        for c0 in range(0, FA, CH):
            c1 = min(c0 + CH, FA)
            if c0 == ORDER:
                if first:
                    wait("c")
                    wait("w2")
                    for bb in range(1, nb):
                        wait(("x", bb))
                    cre = cre_ref[...].astype(f32)
                    cim = cim_ref[...].astype(f32)
                    cp_ref[:, 0:P] = (2.0 * (cre * kr - cim * ki)).astype(bf16)
                    cp_ref[:, P:2 * P] = (-2.0 * (cre * ki + cim * kr)).astype(bf16)
                if b + 1 < nb:
                    norm(b + 1)
            hh_ref[r, c0:c1] = glu(_dnt(xn_ref[r, :], w1_ref[c0:c1, :]),
                                   _dnt(xn_ref[r, :], w3_ref[c0:c1, :]))
        t_ = _dnt(xn_ref[r, :], wt_ref[...])
        hh_ref[r, FA:F] = glu(t_[:, 0:F - FA], t_[:, F - FA:])
        y = _dnt(g_ref[r, :], cp_ref[...])
        y = y + jnp.dot(hh_ref[r, :], w2_ref[...], preferred_element_type=f32)
        for c in range(NC):
            for t in range(S):
                os_ref[c, pl.ds(o + t, 8, stride=S), :] = (
                    y[8 * t:8 * t + 8, 128 * c:128 * c + 128]
                    + res_ref[pl.ds(o + 8 * t, 8), 128 * c:128 * c + 128])
            cp = pltpu.make_async_copy(os_ref.at[c, r], o_hbm.at[r, pl.ds(128 * c, 128)],
                                       osem.at[b * NC + c])
            cp.start()
            outs.append(cp)
    for cp in outs:
        cp.wait()


@jax.jit
def pallas_parallel_sum__ssm_conv_s5__glu_gated_swiglu__prompt_kernel(A_x, A_Lambda_re, A_Lambda_im, A_B_re, A_B_im, A_C_re, A_C_im, A_log_dt, A_Dskip,
           B_x, B_w1, B_w3, B_w2):
    nb = len(BLOCKS)
    vm = pl.BlockSpec(memory_space=pltpu.VMEM)
    hbm = pl.BlockSpec(memory_space=pltpu.HBM)
    out = pl.pallas_call(
        _kernel,
        in_specs=[vm] * 4 + [hbm] * 8,
        out_specs=hbm,
        out_shape=jax.ShapeDtypeStruct((L, D), f32),
        scratch_shapes=[
            pltpu.VMEM((NC, L, 128), bf16), pltpu.VMEM((NC, L, 128), f32),
            pltpu.VMEM((P, D), bf16), pltpu.VMEM((P, D), bf16),
            pltpu.VMEM((D, P), bf16), pltpu.VMEM((D, P), bf16),
            pltpu.VMEM((FA, D), bf16), pltpu.VMEM((FA, D), bf16), pltpu.VMEM((128, D), bf16),
            pltpu.VMEM((F, D), bf16),
            pltpu.VMEM((D, 2 * P), bf16), pltpu.VMEM((L, D), bf16), pltpu.VMEM((L, D), f32),
            pltpu.VMEM((L, 2 * P), f32), pltpu.VMEM((L, 2 * P), bf16), pltpu.VMEM((L, F), bf16),
            pltpu.SemaphoreType.DMA((nb * NC + 12,)), pltpu.SemaphoreType.DMA((nb * NC,)),
        ],
        compiler_params=pltpu.CompilerParams(vmem_limit_bytes=110 * 1024 * 1024),
    )(A_Lambda_re, A_Lambda_im, A_log_dt, A_Dskip, A_x.reshape(L, D),
      A_B_re, A_B_im, A_C_re, A_C_im, B_w1.T, B_w3.T, B_w2)
    return out.reshape(1, L, D)
```
